```python
import os as _os
_os.environ.setdefault("JAX_PLATFORMS", "cpu")
import jax
import jax.numpy as jnp

def _softmax(x, axis=-1):
    return jax.nn.softmax(x, axis=axis)
def _gelu(x):
    return jax.nn.gelu(x, approximate=True)
def _silu(x):
    return jax.nn.silu(x)
def _sigmoid(x):
    return jax.nn.sigmoid(x)
def _layernorm(x, axis=-1, eps=1e-5):
    m = jnp.mean(x, axis=axis, keepdims=True)
    v = jnp.var(x, axis=axis, keepdims=True)
    return (x - m) / jnp.sqrt(v + eps)
def _scatter_add(tgt, idx, src, axis=0):
    return tgt.at[idx].add(src)
def _segment_sum(src, seg, n):
    return jax.ops.segment_sum(src, seg, n)
class _Rng:
    def __init__(self, key):
        self._k = key
    def _next(self):
        self._k, sub = jax.random.split(self._k)
        return sub
    def normal(self, shape):
        return jax.random.normal(self._next(), shape, dtype=jnp.bfloat16)
    def randint(self, lo, hi, shape):
        return jax.random.randint(self._next(), shape, lo, hi, dtype=jnp.int32)
    def uniform(self, shape, lo=0.0, hi=1.0):
        return jax.random.uniform(self._next(), shape, jnp.bfloat16, lo, hi)
    def permutation(self, n):
        return jax.random.permutation(self._next(), n)


kernel_name = 'gated_mix__compressed_kv_cla__ssm_conv_h3__prompt'

def setup_inputs():
    _rng = _Rng(jax.random.key(int.from_bytes(__import__("os").urandom(4), "little")))
    _w = (lambda a: (lambda t: t.astype(jnp.bfloat16) if jnp.issubdtype(t.dtype, jnp.floating) else t)(jnp.asarray(a)))
    def _A_setup():
        B, H, Sq, Sk, D, M = 1, 32, 2048, 2048, 128, 1024
        Dc = 4 * D
        return {
            "x": _w((lambda *s: _rng.normal(s) * 0.05)(B, Sq, M)),
            "c_kv": _w((lambda *s: _rng.normal(s) * 0.8)(B, Sk, Dc)),
            "w_q": _w((lambda *s: _rng.normal(s) * 3.2)(M, H, D) * (M ** -0.5)),
            "w_uk": _w((lambda *s: _rng.normal(s) * 3.2)(Dc, H, D) * (Dc ** -0.5)),
            "w_uv": _w((lambda *s: _rng.normal(s) * 0.8)(Dc, H, D) * (Dc ** -0.5)),
            "w_o": _w((lambda *s: _rng.normal(s) * 0.8)(H, D, M) * ((H * D) ** -0.5)),
        }
    _A_in = _A_setup()

    def _B_setup():
        B, S, D = 1, 2048, 1024
        ks = 4
        return {
            "q": _w((lambda *s: _rng.normal(s) * 0.05)(B, S, D)),
            "k": _w((lambda *s: _rng.normal(s) * 0.8)(B, S, D)),
            "v": _w((lambda *s: _rng.normal(s) * 0.8)(B, S, D)),
            "shift_k": _w((lambda *s: _rng.normal(s) * 0.8)(D, ks) * 0.5),
            "ssm_k": _w((lambda *s: _rng.normal(s) * 0.8)(D, S) * (1.0 / S ** 0.5)),
            "ssm_D": _w((lambda *s: _rng.normal(s) * 0.8)(D)),
        }
    _B_in = _B_setup()

    return {
        "A_x": _A_in["x"],
        "A_c_kv": _A_in["c_kv"],
        "A_w_q": _A_in["w_q"],
        "A_w_uk": _A_in["w_uk"],
        "A_w_uv": _A_in["w_uv"],
        "A_w_o": _A_in["w_o"],
        "B_q": _B_in["q"],
        "B_k": _B_in["k"],
        "B_v": _B_in["v"],
        "B_shift_k": _B_in["shift_k"],
        "B_ssm_k": _B_in["ssm_k"],
        "B_ssm_D": _B_in["ssm_D"],
        "gate_w": _w((lambda *s: _rng.normal(s) * 0.05)(1024) * 16.0),
    }

def reference(A_x, A_c_kv, A_w_q, A_w_uk, A_w_uv, A_w_o, B_q, B_k, B_v, B_shift_k, B_ssm_k, B_ssm_D, gate_w):
    def _A_ref(x, c_kv, w_q, w_uk, w_uv, w_o):
        B, Sq, M = x.shape[0], x.shape[1], x.shape[2]
        Sk = c_kv.shape[1]
        H, D = w_q.shape[1], w_q.shape[2]
        q = jnp.einsum("bqm,mhd->bhqd", x, w_q)
        k = jnp.einsum("bkc,chd->bhkd", c_kv, w_uk)
        v = jnp.einsum("bkc,chd->bhkd", c_kv, w_uv)
        scores = jnp.einsum("bhqd,bhkd->bhqk", q, k) * (D ** -0.5)
        off = Sk - Sq
        qi = jnp.arange(Sq)[:, None]
        kj = jnp.arange(Sk)[None, :]
        cmask = kj <= (qi + off)
        scores = jnp.where(cmask[None, None], scores, -1e9)
        p = _softmax(scores, axis=-1)
        ctx = jnp.einsum("bhqk,bhkd->bhqd", p, v)
        return jnp.einsum("bhqd,hdm->bqm", ctx, w_o)

    def _B_ref(q, k, v, shift_k, ssm_k, ssm_D):
        B, S, D = q.shape
        ks = shift_k.shape[-1]
        k_pad = jnp.pad(k, ((0, 0), (ks - 1, 0), (0, 0)))
        k_shift = jnp.zeros_like(k)
        for t in range(ks):
            k_shift = k_shift + k_pad[:, t:t + S, :] * shift_k[:, ks - 1 - t][None, None, :]
        kv = k_shift * v
        L = 2 * S
        kv_pad = jnp.pad(kv, ((0, 0), (0, S), (0, 0)))
        kf_pad = jnp.pad(ssm_k, ((0, 0), (0, S)))
        kv_f = (lambda x, axes=(-2,-1): jnp.fft.rfft2(x.astype(jnp.float32), axes=axes))(kv_pad[:, None, :, :], axes=(1, 2))
        kf_f = (lambda x, axes=(-2,-1): jnp.fft.rfft2(x.astype(jnp.float32), axes=axes))(kf_pad[:, None, :], axes=(1, 2))
        kf_f = (lambda x, *d: x.transpose(*d))(kf_f, 1, 2, 0)
        y_f = kv_f * kf_f[None, :, :, :]
        y = (lambda x, s, axes=(-2,-1): jnp.fft.irfft2(x, s=s, axes=axes).astype(jnp.bfloat16))(y_f, (1, L), axes=(1, 2))[:, 0, :S, :]
        y = y + kv * ssm_D[None, None, :]
        return q * y

    x = A_x
    g = _sigmoid((x * gate_w).sum(-1, keepdims=True))
    a = _A_ref(x, A_c_kv, A_w_q, A_w_uk, A_w_uv, A_w_o)
    b = _B_ref(x, B_k, B_v, B_shift_k, B_ssm_k, B_ssm_D)
    return g * a + (1 - g) * b
```

```python
import math

import jax
import jax.numpy as jnp
from jax import lax
import jax.experimental.pallas as pl
import jax.experimental.pallas.tpu as pltpu

S, M, C, H, D = 2048, 1024, 512, 32, 128
T = 128
NB = S // T
NCB = M // 128
F32, BF16, U32 = jnp.float32, jnp.bfloat16, jnp.uint32
NT = (((1,), (1,)), ((), ()))
QSCALE = D ** -0.5 * math.log2(math.e)
LOOK = 1
PCH = 2
OCH = 1
IB = 4
XCH = 4


def _dot(a, b):
    return jnp.dot(a, b, preferred_element_type=F32)


def _dot_nt(a, b):
    return lax.dot_general(a, b, NT, preferred_element_type=F32)


def _kernel(x_hbm, ckv_hbm, wq_hbm, wuk_hbm, wuv_hbm, wo_hbm, k_hbm, v_hbm,
            shift_ref, h_hbm, d_ref, gw_ref, out_hbm,
            x_s, ckv_s, wq_s, wuk_s, wuv_s, wo_s, bk_s, bv_s, h_s,
            w_s, q_s, k_s, v_s, ctx_s, g_s, f_s, finv_s, par_s,
            kpad_s, kv_s, uf_s, hf_s, yf_s, a_s, o_s,
            sem_x, sem_c, sem_w, sem_b, sem_o):
    wq_u, wuk_u, wuv_u = (r.bitcast(U32) for r in (wq_hbm, wuk_hbm, wuv_hbm))
    rows = S // XCH

    def w_copies(p):
        return [pltpu.make_async_copy(wuk_u.at[:, p, :], wuk_s.at[p], sem_w.at[3 * p]),
                pltpu.make_async_copy(wuv_u.at[:, p, :], wuv_s.at[p], sem_w.at[3 * p + 1]),
                pltpu.make_async_copy(wq_u.at[:, p, :], wq_s.at[p], sem_w.at[3 * p + 2])]

    c_copies = [pltpu.make_async_copy(ckv_hbm.at[pl.ds(r * rows, rows), :],
                                      ckv_s.at[pl.ds(r * rows, rows), :], sem_c.at[r])
                for r in range(XCH)]
    x_copies = [[pltpu.make_async_copy(x_hbm.at[pl.ds(r * rows, rows), pl.ds(c * 128, 128)],
                                       x_s.at[c, pl.ds(r * rows, rows), :], sem_x.at[r * NCB + c])
                 for c in range(NCB)] for r in range(XCH)]
    b_copies = []
    for c in range(NCB):
        cs = pl.ds(c * 128, 128)
        b_copies += [
            pltpu.make_async_copy(k_hbm.at[:, cs], bk_s.at[c], sem_b.at[4 * c]),
            pltpu.make_async_copy(v_hbm.at[:, cs], bv_s.at[c], sem_b.at[4 * c + 1]),
            pltpu.make_async_copy(h_hbm.at[cs, :], h_s.at[c], sem_b.at[4 * c + 2]),
            pltpu.make_async_copy(wo_hbm.at[:, cs], wo_s.at[c], sem_b.at[4 * c + 3]),
        ]

    w0 = w_copies(0)
    w0[0].start()
    w0[1].start()
    for cp in c_copies:
        cp.start()
    w0[2].start()
    for cps in x_copies:
        for cp in cps:
            cp.start()

    def dft(shape, fdim):
        r = lax.broadcasted_iota(jnp.int32, shape, fdim)
        n = lax.broadcasted_iota(jnp.int32, shape, 1 - fdim)
        g = ((r >> 4) << 3) + (r & 7)
        ph = ((4 * g + 1) * n - ((r >> 3) & 1) * 128) & 511
        ph = jnp.where(ph > 256, ph - 512, ph)
        return jnp.cos(ph.astype(F32) * (math.pi / 256))

    f_s[...] = dft((2 * T, T), 0).astype(BF16)
    finv_s[...] = (dft((T, 2 * T), 1) * (1.0 / T)).astype(BF16)
    shift = shift_ref[...].astype(F32)
    dvec = d_ref[...].astype(F32)
    for c in range(NCB):
        for t in range(4):
            par_s[c, t] = jnp.broadcast_to(shift[t:t + 1, c * 128:(c + 1) * 128], (8, 128))
        par_s[c, 4] = jnp.broadcast_to(dvec[c:c + 1, :], (8, 128))
    kpad_s[0:8, :] = jnp.zeros((8, 128), F32)

    def unpack(words, odd):
        sh = (16 * (1 - odd)).astype(U32) if not isinstance(odd, int) else 16 * (1 - odd)
        return pltpu.bitcast((words << sh) & U32(0xFFFF0000), F32).astype(BF16)

    def load_wkv(h):
        w_s[M:M + C, :] = unpack(wuk_s[h // 2], h % 2)
        w_s[M + C:, :] = unpack(wuv_s[h // 2], h % 2)

    def load_wq(h):
        w_s[0:M, :] = unpack(wq_s[h // 2], h % 2)

    def proj_kv(r0, n):
        c = ckv_s[r0:r0 + n, :]
        k_s[r0:r0 + n, :] = _dot(c, w_s[M:M + C, :]).astype(BF16)
        v_s[r0:r0 + n, :] = _dot(c, w_s[M + C:, :]).astype(BF16)

    def proj_q(r0, n):
        x = jnp.concatenate([x_s[c, r0:r0 + n, :] for c in range(NCB)], axis=1)
        q_s[r0:r0 + n, :] = (_dot(x, w_s[0:M, :]) * QSCALE).astype(BF16)

    w0[0].wait()
    w0[1].wait()
    load_wkv(0)
    for r in range(XCH):
        c_copies[r].wait()
        proj_kv(r * rows, rows)
    w0[2].wait()
    load_wq(0)
    gw = gw_ref[...].astype(F32)
    for r in range(XCH):
        for cp in x_copies[r]:
            cp.wait()
        if r == XCH - 1:
            for p in range(1, H // 2):
                for cp in w_copies(p):
                    cp.start()
            for cp in b_copies:
                cp.start()
        proj_q(r * rows, rows)
        acc = x_s[0, r * rows:(r + 1) * rows, :].astype(F32) * gw[0:1, :]
        for c in range(1, NCB):
            acc = acc + x_s[c, r * rows:(r + 1) * rows, :].astype(F32) * gw[c:c + 1, :]
        z = jnp.sum(acc, axis=1, keepdims=True)
        g_s[r * rows:(r + 1) * rows, :] = jax.nn.sigmoid(jnp.broadcast_to(z, (rows, 128)))

    def attention(h, filler):
        tri = (lax.broadcasted_iota(jnp.int32, (T, T), 1)
               <= lax.broadcasted_iota(jnp.int32, (T, T), 0))

        def scores(i):
            n = (i + 1) * T
            s = _dot_nt(q_s[i * T:n, :], k_s[0:n, :])
            sd = jnp.where(tri, s[:, n - T:], -1e30)
            return jnp.concatenate([s[:, :n - T], sd], axis=1) if i else sd

        def context(i, s):
            n = (i + 1) * T
            p = jnp.exp2(s - jnp.max(s, axis=1, keepdims=True))
            l = jnp.sum(p, axis=1, keepdims=True)
            o = _dot(p.astype(BF16), v_s[0:n, :])
            ctx_s[h, i * T:n, :] = (o * pltpu.reciprocal(l, approx=True)).astype(BF16)

        order = list(range(NB))[::-1]
        pend = {}
        for t in range(NB + LOOK):
            if t < NB:
                pend[order[t]] = scores(order[t])
            if t >= LOOK:
                i = order[t - LOOK]
                context(i, pend.pop(i))
                filler(i)

    def head_body(h, carry):
        nxt = h + 1

        @pl.when(nxt % 2 == 0)
        def _():
            p = nxt // 2
            pltpu.make_async_copy(wuk_s.at[p], wuk_s.at[p], sem_w.at[3 * p]).wait()
            pltpu.make_async_copy(wuv_s.at[p], wuv_s.at[p], sem_w.at[3 * p + 1]).wait()
            pltpu.make_async_copy(wq_s.at[p], wq_s.at[p], sem_w.at[3 * p + 2]).wait()

        load_wkv(nxt)
        load_wq(nxt)

        def filler(i):
            if i % PCH == 0:
                proj_q(i * T, PCH * T)
                proj_kv(i * T, PCH * T)

        attention(h, filler)
        return carry

    lax.fori_loop(0, H - 1, head_body, 0)
    attention(H - 1, lambda i: None)

    for cp in b_copies:
        cp.wait()

    def out_copy(c):
        return pltpu.make_async_copy(
            o_s.at[c], out_hbm.at[:, pl.ds(pl.multiple_of(c * 128, 128), 128)], sem_o.at[c])

    def chan_body(c, carry):
        def oproj(i):
            r0, n = i * T, OCH * T
            ctx = jnp.concatenate([ctx_s[hh, r0:r0 + n, :] for hh in range(H)], axis=1)
            return _dot(ctx, wo_s[c])

        f = f_s[...]
        prev = None
        for d in range(NB):
            cur = _dot_nt(f, h_s[c, :, d * T:(d + 1) * T]).reshape(16, 2, 8, 128)
            if prev is None:
                re, im = cur[:, 0], cur[:, 1]
            else:
                re, im = cur[:, 0] + prev[:, 1], cur[:, 1] - prev[:, 0]
            hf_s[:, 0, d] = re
            hf_s[:, 1, d] = im
            prev = cur

        kpad_s[8:, :] = bk_s[c].astype(F32)
        for j in range(NB):
            ks = None
            for t in range(4):
                term = (kpad_s[8 + j * T - t:8 + (j + 1) * T - t, :].reshape(16, 8, 128)
                        * par_s[c, t][None])
                ks = term if ks is None else ks + term
            kv = ks.reshape(T, 128) * bv_s[c, j * T:(j + 1) * T, :].astype(F32)
            kv_s[j * T:(j + 1) * T, :] = kv
            u = _dot(f, kv.astype(BF16)).reshape(16, 2, 8, 128)
            uf_s[:, 0, j] = u[:, 0]
            uf_s[:, 1, j] = u[:, 1]

        def conv(fg):
            for i0 in range(0, NB, IB):
                ar = ai = None
                for j in range(i0 + 1):
                    hr, hi = hf_s[fg, 0, i0 - j:i0 - j + IB], hf_s[fg, 1, i0 - j:i0 - j + IB]
                    ur, ui = uf_s[fg, 0, j][None], uf_s[fg, 1, j][None]
                    tr, ti = hr * ur - hi * ui, hr * ui + hi * ur
                    ar, ai = (tr, ti) if ar is None else (ar + tr, ai + ti)
                ar, ai = [ar[n] for n in range(IB)], [ai[n] for n in range(IB)]
                for j in range(i0 + 1, i0 + IB):
                    ur, ui = uf_s[fg, 0, j], uf_s[fg, 1, j]
                    for i in range(j, i0 + IB):
                        hr, hi = hf_s[fg, 0, i - j], hf_s[fg, 1, i - j]
                        ar[i - i0] = ar[i - i0] + (hr * ur - hi * ui)
                        ai[i - i0] = ai[i - i0] + (hr * ui + hi * ur)
                for n in range(IB):
                    yf_s[i0 + n, fg * 16:(fg + 1) * 16, :] = jnp.concatenate(
                        [ar[n], ai[n]], axis=0).astype(BF16)

        nch = NB // OCH
        for ch in range(nch - 1):
            a_s[ch * OCH * T:(ch + 1) * OCH * T, :] = oproj(ch * OCH)
        for fg in range(16):
            conv(fg)

        finv = finv_s[...]
        for i in range(NB):
            rs = slice(i * T, (i + 1) * T)
            y = _dot(finv, yf_s[i])
            y = y + (kv_s[rs, :].reshape(16, 8, 128) * par_s[c, 4][None]).reshape(T, 128)
            kv_s[rs, :] = y * x_s[c, rs, :].astype(F32)
        a_last = oproj((nch - 1) * OCH)
        for i in range(NB):
            rs = slice(i * T, (i + 1) * T)
            if i < (nch - 1) * OCH:
                a = a_s[rs, :]
            else:
                a = a_last[(i - (nch - 1) * OCH) * T:(i + 1 - (nch - 1) * OCH) * T]
            g = g_s[rs, :]
            o_s[c, rs, :] = (g * a + (1.0 - g) * kv_s[rs, :]).astype(BF16)
        out_copy(c).start()
        return carry

    lax.fori_loop(0, NCB, chan_body, 0)
    for c in range(NCB):
        out_copy(c).wait()


@jax.jit
def pallas_gated_mix__compressed_kv_cla__ssm_conv_h3__prompt_kernel(
        A_x, A_c_kv, A_w_q, A_w_uk, A_w_uv, A_w_o, B_q, B_k, B_v,
        B_shift_k, B_ssm_k, B_ssm_D, gate_w):
    del B_q
    hbm = pl.BlockSpec(memory_space=pl.ANY)
    vmem = pl.BlockSpec(memory_space=pltpu.VMEM)
    V = pltpu.VMEM
    out = pl.pallas_call(
        _kernel,
        out_shape=jax.ShapeDtypeStruct((S, M), BF16),
        in_specs=[hbm] * 8 + [vmem, hbm, vmem, vmem],
        out_specs=hbm,
        scratch_shapes=[
            V((NCB, S, 128), BF16),
            V((S, C), BF16),
            V((H // 2, M, D), U32),
            V((H // 2, C, D), U32),
            V((H // 2, C, D), U32),
            V((NCB, H * D, 128), BF16),
            V((NCB, S, 128), BF16),
            V((NCB, S, 128), BF16),
            V((NCB, 128, S), BF16),
            V((M + 2 * C, D), BF16),
            V((S, D), BF16),
            V((S, D), BF16),
            V((S, D), BF16),
            V((H, S, D), BF16),
            V((S, 128), F32),
            V((2 * T, T), BF16),
            V((T, 2 * T), BF16),
            V((NCB, 5, 8, 128), F32),
            V((S + 8, 128), F32),
            V((S, 128), F32),
            V((16, 2, NB, 8, 128), F32),
            V((16, 2, NB, 8, 128), F32),
            V((NB, 2 * T, 128), BF16),
            V((S, 128), F32),
            V((NCB, S, 128), BF16),
            pltpu.SemaphoreType.DMA((XCH * NCB,)),
            pltpu.SemaphoreType.DMA((XCH,)),
            pltpu.SemaphoreType.DMA((3 * H // 2,)),
            pltpu.SemaphoreType.DMA((4 * NCB,)),
            pltpu.SemaphoreType.DMA((NCB,)),
        ],
        compiler_params=pltpu.CompilerParams(vmem_limit_bytes=110 * 2 ** 20),
    )(A_x.reshape(S, M), A_c_kv.reshape(S, C), A_w_q, A_w_uk, A_w_uv,
      A_w_o.reshape(H * D, M), B_k.reshape(S, M), B_v.reshape(S, M),
      B_shift_k.T, B_ssm_k, B_ssm_D.reshape(NCB, 128), gate_w.reshape(NCB, 128))
    return out.reshape(1, S, M)
```

```python
import math

import jax
import jax.numpy as jnp
from jax import lax
import jax.experimental.pallas as pl
import jax.experimental.pallas.tpu as pltpu

S, M, C, H, D = 2048, 1024, 512, 32, 128
T = 128
W = T // 2
NB = S // T
NCB = M // 128
NFG = T // 8
F32, BF16, U32 = jnp.float32, jnp.bfloat16, jnp.uint32
QSCALE = D ** -0.5 * math.log2(math.e)

CB, NFIRST = 3, 4
REST = NB - CB * NFIRST
X_SPLIT = 10
W_SPLIT = 4
O_HR, O_HI, O_UR, O_UI = S, 2 * S, 3 * S, 4 * S


def _dot(a, b):
    return jnp.dot(a, b, preferred_element_type=F32)


def _dot_nt(a, b):
    return lax.dot_general(a, b, (((1,), (1,)), ((), ())), preferred_element_type=F32)


def _bf(words):
    return pltpu.bitcast(words, BF16)


def _words(val):
    return pltpu.bitcast(val.astype(BF16), U32)


def _blk(i):
    return slice(i * T, (i + 1) * T)


def _wblk(i):
    return slice(i * W, (i + 1) * W)


def _lanes(c):
    return pl.ds(pl.multiple_of(c * 128, 128), 128)


def _plan(refill, hurry=0):
    delay = {"q": 0, "s": 1, "f": 4, "c": 2, "k": 2, "v": 2}
    steps = []
    for n in range(NB):
        i = NB - 1 - n
        for pos, op in enumerate("qsfckv"):
            if op in "kv" and i >= refill:
                continue
            t = NB - 1 - hurry if op in "qs" and i < hurry else n
            steps.append((t + delay[op], pos, n, op, i))
    return [step[3:] for step in sorted(steps)]


def _kernel(x_hbm, ckv_hbm, wq_hbm, wuk_hbm, wuv_hbm, wo_hbm, k_hbm, v_hbm,
            shift_hbm, h_hbm, d_hbm, gw_hbm, out_hbm,
            x_s, ckv_s, wq_s, wuk_s, wuv_s, wo_s, bk_s, bv_s, h_s, shift_s, d_s, gw_s,
            w0_s, w_s, v0_s, v_s, ctx_s, g_s, f_s, finv_s, par_s, a_s, spec_s, o_s,
            zero_s, sems):
    x_u, ckv_u, wq_u, wuk_u, wuv_u, wo_u, k_u, v_u, out_u = (
        r.bitcast(U32) for r in
        (x_hbm, ckv_hbm, wq_hbm, wuk_hbm, wuv_hbm, wo_hbm, k_hbm, v_hbm, out_hbm))
    k_s, k0_s = ctx_s.at[H], ctx_s.at[H + 1]
    zero_s[0] = 0

    def w_copies(p):
        kv, q = (0, 1) if p == 0 else (2, 2) if p < W_SPLIT else (3, 3)
        return [pltpu.make_async_copy(wuk_u.at[:, p, :], wuk_s.at[p], sems.at[kv]),
                pltpu.make_async_copy(wuv_u.at[:, p, :], wuv_s.at[p], sems.at[kv]),
                pltpu.make_async_copy(wq_u.at[:, p, :], wq_s.at[p], sems.at[q])]

    def row_copy(src, dst, rows, sem):
        return pltpu.make_async_copy(src.at[rows, :], dst.at[rows, :], sems.at[sem])

    def c_rows(n):
        return pl.ds(pl.multiple_of((NB - CB * (n + 1)) * W, W), CB * W)

    def c_copy(n):
        return row_copy(ckv_u, ckv_s, c_rows(n), 10 + n)

    c_rest = row_copy(ckv_u, ckv_s, pl.ds(0, REST * W), 7)
    x_high = row_copy(x_u, x_s, pl.ds(X_SPLIT * W, (NB - X_SPLIT) * W), 8)
    x_low = row_copy(x_u, x_s, pl.ds(0, X_SPLIT * W), 9)
    gw_copy = pltpu.make_async_copy(gw_hbm, gw_s, sems.at[6])
    mix_copies = [pltpu.make_async_copy(src, dst, sems.at[4]) for src, dst in (
        (shift_hbm, shift_s), (d_hbm, d_s), (h_hbm, h_s))]
    for c in range(NCB):
        mix_copies += [
            pltpu.make_async_copy(src.at[:, pl.ds(c * 128, 128)], dst, sems.at[4])
            for src, dst in ((k_u, bk_s.at[pl.ds(S + c * (S // 2), S // 2), :]),
                             (v_u, bv_s.at[c]), (wo_u, wo_s.at[c]))]

    w_first = w_copies(0)
    for cp in (w_first[:2] + [c_copy(n) for n in range(NFIRST)]
               + [c_rest, w_first[2], x_high, x_low, gw_copy]
               + [cp for p in range(1, H // 2) for cp in w_copies(p)]):
        cp.start()

    def phasor(rows, step, first):
        r = lax.broadcasted_iota(jnp.int32, (rows, T), 0)
        n = lax.broadcasted_iota(jnp.int32, (rows, T), 1)
        ang = (((step * r + first) * n) & (4 * T - 1)).astype(F32) * (math.pi / (2 * T))
        return jnp.cos(ang), jnp.sin(ang)

    ca, sa = phasor(8, 4, 1)
    cb, sb = phasor(NFG, 32, 0)
    fwd = []
    for fg in range(NFG):
        cf, sf = cb[fg:fg + 1, :], sb[fg:fg + 1, :]
        fwd += [ca * cf - sa * sf, sa * cf + ca * sf]
    fwd = jnp.concatenate(fwd, axis=0)
    f_s[...] = _words(fwd)
    finv_s[...] = _words(fwd.T * (1.0 / T))

    wq_rows, wk_rows, wv_rows = (
        slice(0, M // 2), slice(M // 2, (M + C) // 2), slice((M + C) // 2, M // 2 + C))

    def head_weights(pair, odd):
        if isinstance(odd, int):
            half = pair & U32(0xFFFF0000) if odd else pair << 16
        else:
            half = (pair << (16 - 16 * odd).astype(U32)) & U32(0xFFFF0000)
        return _words(pltpu.bitcast(half, F32))

    def load_wkv(w_ref, p, odd):
        w_ref[wk_rows, :] = head_weights(wuk_s[p], odd)
        w_ref[wv_rows, :] = head_weights(wuv_s[p], odd)

    def load_wq(p, odd):
        w_s[wq_rows, :] = head_weights(wq_s[p], odd)

    def up_project(dst, w_ref, w_rows, rows):
        dst[rows, :] = _words(_dot(_bf(ckv_s[rows, :]), _bf(w_ref[w_rows, :])))

    def gate_rows(h):
        rows = S // H
        gw = gw_s[...].astype(F32)
        acc = None
        for c in range(NCB):
            xw = x_s[pl.ds(pl.multiple_of(h * (rows // 2), rows // 2), rows // 2),
                     c * 128:(c + 1) * 128]
            term = _bf(xw).astype(F32) * gw[c:c + 1, :]
            acc = term if acc is None else acc + term
        z = jnp.sum(acc, axis=1, keepdims=True)
        g_s[pl.ds(pl.multiple_of(h * rows, rows), rows), :] = jax.nn.sigmoid(
            jnp.broadcast_to(z, (rows, 128)))

    def attention(h, k_ref, v_ref, plan, after_q, before_q=None):
        causal = (lax.broadcasted_iota(jnp.int32, (T, T), 1)
                  <= lax.broadcasted_iota(jnp.int32, (T, T), 0))
        val = {}
        for op, i in plan:
            n = (i + 1) * T
            if op == "q":
                if before_q is not None:
                    before_q(i)
                q = _dot(_bf(x_s[_wblk(i), :]), _bf(w_s[wq_rows, :]))
                val[i] = (q * QSCALE).astype(BF16)
                if i == 0:
                    after_q()
            elif op == "s":
                s = _dot_nt(val[i], _bf(k_ref[0:n // 2, :]))
                diag = jnp.where(causal, s[:, n - T:], -1e30)
                val[i] = jnp.concatenate([s[:, :n - T], diag], axis=1) if i else diag
            elif op == "c":
                p = jnp.exp2(val[i] - jnp.max(val[i], axis=1, keepdims=True))
                l = jnp.sum(p, axis=1, keepdims=True)
                o = _dot(p.astype(BF16), _bf(v_ref[0:n // 2, :]))
                val[i] = _words(o * pltpu.reciprocal(l, approx=True))
            elif op == "f":
                ctx_s[h, _wblk(i), :] = val.pop(i)
            elif op == "k":
                up_project(k_s, w_s, wk_rows, _wblk(i))
            else:
                up_project(v_s, w_s, wv_rows, _wblk(i))

    w_first[0].wait()
    w_first[1].wait()
    load_wkv(w0_s, 0, 0)
    load_wkv(w_s, 0, 1)

    def first_body(n, carry):
        c_copy(n).wait()
        up_project(k0_s, w0_s, wk_rows, c_rows(n))
        up_project(v0_s, w0_s, wv_rows, c_rows(n))
        up_project(k_s, w_s, wk_rows, c_rows(n))
        up_project(v_s, w_s, wv_rows, c_rows(n))
        return carry

    lax.fori_loop(0, NFIRST, first_body, 0)
    c_rest.wait()
    w_first[2].wait()
    load_wq(0, 0)
    up_project(k0_s, w0_s, wk_rows, slice(0, REST * W))
    up_project(v0_s, w0_s, wv_rows, slice(0, REST * W))

    def wait_x(i):
        if i == NB - 1:
            x_high.wait()
        if i == X_SPLIT - 1:
            x_low.wait()
            gw_copy.wait()

    def after_first():
        load_wq(0, 1)
        gate_rows(0)

    attention(zero_s[0], k0_s, v0_s, _plan(REST), after_first, wait_x)
    for p in range(1, W_SPLIT):
        for cp in w_copies(p):
            cp.wait()
    for cp in mix_copies:
        cp.start()

    def head_body(h, carry):
        nxt = h + 1

        @pl.when(nxt == 2 * W_SPLIT)
        def _():
            for p in range(W_SPLIT, H // 2):
                for cp in w_copies(p):
                    cp.wait()

        def after_q():
            load_wq(nxt >> 1, nxt & 1)
            gate_rows(h)

        load_wkv(w_s, nxt >> 1, nxt & 1)
        attention(h, k_s, v_s, _plan(NB), after_q)
        return carry

    lax.fori_loop(1, H - 1, head_body, 0)

    for cp in mix_copies:
        cp.wait()
    shift = shift_s[...].astype(F32)
    skip_w = d_s[...].astype(F32)
    for c in range(NCB):
        for t in range(4):
            par_s[c, t] = jnp.broadcast_to(shift[t:t + 1, c * 128:(c + 1) * 128], (8, 128))
        par_s[c, 4] = jnp.broadcast_to(skip_w[c:c + 1, :], (8, 128))
    attention(zero_s[0] + (H - 1), k_s, v_s, _plan(0, 2), lambda: gate_rows(H - 1))

    def out_copy(c):
        return pltpu.make_async_copy(o_s.at[c], out_u.at[:, _lanes(c)], sems.at[5])

    def channel_body(c, carry):
        row0 = pl.multiple_of(zero_s[0] * 8, 8)

        def vregs(base, fg, j, n=1):
            return pl.ds(base + (fg * NB + j) * 8, 8 * n)

        def out_project(i):
            ctx = jnp.concatenate([_bf(ctx_s[h, _wblk(i), :]) for h in range(H)], axis=1)
            return _dot(ctx, _bf(wo_s[c]))

        def short_conv(j, before):
            k = _bf(bk_s[pl.ds(pl.multiple_of(S + c * (S // 2) + j * 8, 8), 8), :]).astype(F32)
            ext = jnp.concatenate([before, k], axis=0)
            acc = None
            for t in range(4):
                term = ext[8 - t:24 - t].reshape(2, 8, 128) * par_s[c, t][None]
                acc = term if acc is None else acc + term
            kv = acc.reshape(16, 128) * _bf(bv_s[c, j * 8:(j + 1) * 8, :]).astype(F32)
            bk_s[pl.ds(pl.multiple_of(row0 + j * 16, 8), 16), :] = pltpu.bitcast(kv, U32)
            return k[8:]

        def kv_block(j):
            return pltpu.bitcast(bk_s[_blk(j), :], F32)

        def signal_spectrum(j):
            u = _dot(_bf(f_s[...]), kv_block(j).astype(BF16)).reshape(NFG, 2, 8, 128)
            for fg in range(NFG):
                spec_s[vregs(O_UR, fg, j), :] = u[fg, 0]
                spec_s[vregs(O_UI, fg, j), :] = u[fg, 1]

        def filter_spectrum(d, prev):
            cur = _dot_nt(_bf(f_s[...]), h_s[_lanes(c), _blk(d)]).reshape(NFG, 2, 8, 128)
            re, im = cur[:, 0], cur[:, 1]
            if prev is not None:
                re, im = re + prev[:, 1], im - prev[:, 0]
            for fg in range(NFG):
                spec_s[vregs(O_HR, fg, d), :] = re[fg]
                spec_s[vregs(O_HI, fg, d), :] = im[fg]
            return cur

        def block_conv(fg, i):
            yr = yi = None
            for j in range(i + 1):
                hr = spec_s[vregs(O_HR, fg, i - j, 2), :].reshape(2, 8, 128)
                hi = spec_s[vregs(O_HI, fg, i - j, 2), :].reshape(2, 8, 128)
                ur = spec_s[vregs(O_UR, fg, j), :][None]
                ui = spec_s[vregs(O_UI, fg, j), :][None]
                tr, ti = hr * ur - hi * ui, hr * ui + hi * ur
                yr, yi = (tr, ti) if yr is None else (yr + tr, yi + ti)
            ur, ui = spec_s[vregs(O_UR, fg, i + 1), :], spec_s[vregs(O_UI, fg, i + 1), :]
            hr, hi = spec_s[vregs(O_HR, fg, 0), :], spec_s[vregs(O_HI, fg, 0), :]
            pairs = ((yr[0], yi[0]),
                     (yr[1] + (hr * ur - hi * ui), yi[1] + (hr * ui + hi * ur)))
            for n, pair in enumerate(pairs):
                row = pl.multiple_of(row0 + ((i + n) * NFG + fg) * 8, 8)
                spec_s[pl.ds(row, 8), :] = pltpu.bitcast(
                    jnp.concatenate(pair, axis=0).astype(BF16), F32)

        before = jnp.zeros((8, 128), F32)
        for j in range(S // 16):
            before = short_conv(j, before)
        a = {}
        for i in range(NB - 1):
            a[i] = out_project(i)
            if i == 2:
                for j in range(NB):
                    signal_spectrum(j)
            if i == 3:
                prev = None
                for d in range(NB):
                    prev = filter_spectrum(d, prev)
            if i:
                a_s[pl.ds(pl.multiple_of(row0 + (i - 1) * T, 8), T), :] = a.pop(i - 1)
        for fg in range(NFG):
            for i in range(0, NB, 2):
                block_conv(fg, i)
        y = [_dot(_bf(finv_s[...]), _bf(spec_s[_blk(i), :])) for i in range(NB)]
        a[NB - 1] = out_project(NB - 1)
        for i in range(NB):
            g = g_s[_blk(i), :]
            skip = (kv_block(i).reshape(T // 8, 8, 128) * par_s[c, 4][None]).reshape(T, 128)
            b = _bf(x_s[_wblk(i), _lanes(c)]).astype(F32) * (y[i] + skip)
            o_s[c, _wblk(i), :] = _words(
                g * (a[i] if i in a else a_s[_blk(i), :]) + (1.0 - g) * b)
        out_copy(c).start()
        return carry

    lax.fori_loop(0, NCB, channel_body, 0)
    for c in range(NCB):
        out_copy(c).wait()


@jax.jit
def pallas_gated_mix__compressed_kv_cla__ssm_conv_h3__prompt_kernel(
    A_x: jax.Array,
    A_c_kv: jax.Array,
    A_w_q: jax.Array,
    A_w_uk: jax.Array,
    A_w_uv: jax.Array,
    A_w_o: jax.Array,
    B_q: jax.Array,
    B_k: jax.Array,
    B_v: jax.Array,
    B_shift_k: jax.Array,
    B_ssm_k: jax.Array,
    B_ssm_D: jax.Array,
    gate_w: jax.Array,
):
    del B_q
    hbm = pl.BlockSpec(memory_space=pl.ANY)
    vmem = pltpu.VMEM
    out = pl.pallas_call(
        _kernel,
        out_shape=jax.ShapeDtypeStruct((S, M), BF16),
        in_specs=[hbm] * 12,
        out_specs=hbm,
        scratch_shapes=[
            vmem((S // 2, M), U32),
            vmem((S // 2, C), U32),
            vmem((H // 2, M, D), U32),
            vmem((H // 2, C, D), U32),
            vmem((H // 2, C, D), U32),
            vmem((NCB, H * D // 2, 128), U32),
            vmem((S + NCB * S // 2, 128), U32),
            vmem((NCB, S // 2, 128), U32),
            vmem((M, S), BF16),
            vmem((4, M), BF16),
            vmem((NCB, 128), BF16),
            vmem((NCB, 128), BF16),
            vmem((M // 2 + C, D), U32),
            vmem((M // 2 + C, D), U32),
            vmem((S // 2, D), U32),
            vmem((S // 2, D), U32),
            vmem((H + 2, S // 2, D), U32),
            vmem((S, 128), F32),
            vmem((T, T), U32),
            vmem((T // 2, 2 * T), U32),
            vmem((NCB, 8, 8, 128), F32),
            vmem((S, 128), F32),
            vmem((5 * S, 128), F32),
            vmem((NCB, S // 2, 128), U32),
            pltpu.SMEM((1,), jnp.int32),
            pltpu.SemaphoreType.DMA((10 + NFIRST,)),
        ],
        compiler_params=pltpu.CompilerParams(vmem_limit_bytes=110 * 2 ** 20),
    )(A_x.reshape(S, M), A_c_kv.reshape(S, C), A_w_q, A_w_uk, A_w_uv,
      A_w_o.reshape(H * D, M), B_k.reshape(S, M), B_v.reshape(S, M),
      B_shift_k.T, B_ssm_k, B_ssm_D.reshape(NCB, 128), gate_w.reshape(NCB, 128))
    return out.reshape(1, S, M)
```

```python
import math

import jax
import jax.numpy as jnp
from jax import lax
import jax.experimental.pallas as pl
import jax.experimental.pallas.tpu as pltpu

S, M, C, H, D = 2048, 1024, 512, 32, 128
T = 128
W = T // 2
NB = S // T
NCB = M // 128
NFG = T // 8
F32, BF16, U32 = jnp.float32, jnp.bfloat16, jnp.uint32
QSCALE = D ** -0.5 * math.log2(math.e)

C_CHUNKS = 8
X_SPLIT = 8
W_SPLIT = 4
OUT_SPLIT = 14
KV_ROWS = 32
O_HR, O_HI, O_UR, O_UI = S, 2 * S, 3 * S, 4 * S


def _dot(a, b):
    return jnp.dot(a, b, preferred_element_type=F32)


def _dot_nt(a, b):
    return lax.dot_general(a, b, (((1,), (1,)), ((), ())), preferred_element_type=F32)


def _bf(words):
    return pltpu.bitcast(words, BF16)


def _words(val):
    return pltpu.bitcast(val.astype(BF16), U32)


def _blk(i):
    return slice(i * T, (i + 1) * T)


def _wblk(i):
    return slice(i * W, (i + 1) * W)


def _lanes(c):
    return pl.ds(pl.multiple_of(c * 128, 128), 128)


def _plan(delays, hurry=0):
    steps = []
    for n in range(NB):
        i = NB - 1 - n
        for pos, (op, delay) in enumerate(delays):
            t = NB - 1 - hurry if op in "qs" and i < hurry else n
            steps.append((t + delay, pos, n, op, i))
    return [step[3:] for step in sorted(steps)]


_REFILL_PLAN = _plan((("s", 2), ("f", 5), ("q", 0), ("k", 3), ("v", 3), ("c", 2)))
_PLAIN_PLAN = _plan((("q", 0), ("s", 1), ("f", 3), ("c", 2)), hurry=2)


def _dft(groups, time):
    def phasor(rows, step, first):
        r = lax.broadcasted_iota(jnp.int32, (rows, T), 0)
        n = time(lax.broadcasted_iota(jnp.int32, (rows, T), 1))
        ang = (((step * r + first) * n) & (4 * T - 1)).astype(F32) * (math.pi / (2 * T))
        return jnp.cos(ang), jnp.sin(ang)

    ca, sa = phasor(8, 4, 1)
    cb, sb = phasor(groups, 32, 0)
    rows = []
    for fg in range(groups):
        cf, sf = cb[fg:fg + 1, :], sb[fg:fg + 1, :]
        rows += [ca * cf - sa * sf, sa * cf + ca * sf]
    return jnp.concatenate(rows, axis=0)


def _kernel(x_hbm, ckv_hbm, wq_hbm, wuk_hbm, wuv_hbm, wo_hbm, k_hbm, v_hbm,
            shift_hbm, h_hbm, d_hbm, gw_hbm, out_hbm,
            x_s, ckv_s, wq_s, wuk_s, wuv_s, wo_s, bk_s, bv_s, h_s, shift_s, d_s, gw_s,
            w0_s, w_s, val_s, ctx_s, g_s, f_s, finv_s, par_s, base_s, gain_s, spec_s,
            o_s, zero_s, sems):
    x_u, ckv_u, wq_u, wuk_u, wuv_u, wo_u, k_u, v_u, out_u = (
        r.bitcast(U32) for r in
        (x_hbm, ckv_hbm, wq_hbm, wuk_hbm, wuv_hbm, wo_hbm, k_hbm, v_hbm, out_hbm))
    k_s, k0_s = ctx_s.at[H], ctx_s.at[H + 1]
    v_s, v0_s = val_s.at[0], val_s.at[1]
    zero_s[0] = 0

    def w_copies(p):
        kv, q = (0, 1) if p == 0 else (2, 2) if p < W_SPLIT else (3, 3)
        return [pltpu.make_async_copy(wuk_u.at[:, p, :], wuk_s.at[p], sems.at[kv]),
                pltpu.make_async_copy(wuv_u.at[:, p, :], wuv_s.at[p], sems.at[kv]),
                pltpu.make_async_copy(wq_u.at[:, p, :], wq_s.at[p], sems.at[q])]

    def row_copy(src, dst, rows, sem):
        return pltpu.make_async_copy(src.at[rows, :], dst.at[rows, :], sems.at[sem])

    def c_rows(n):
        rows = S // 2 // C_CHUNKS
        return pl.ds(pl.multiple_of(n * rows, rows), rows)

    def c_copy(n):
        return row_copy(ckv_u, ckv_s, c_rows(n), 9 + n)

    gw_copy = pltpu.make_async_copy(gw_hbm, gw_s, sems.at[6])
    x_high = row_copy(x_u, x_s, pl.ds(X_SPLIT * W, (NB - X_SPLIT) * W), 7)
    x_low = row_copy(x_u, x_s, pl.ds(0, X_SPLIT * W), 8)
    mix_copies = [pltpu.make_async_copy(src, dst, sems.at[4]) for src, dst in (
        (shift_hbm, shift_s), (d_hbm, d_s), (h_hbm, h_s))]
    for c in range(NCB):
        mix_copies += [
            pltpu.make_async_copy(src.at[:, pl.ds(c * 128, 128)], dst, sems.at[4])
            for src, dst in ((k_u, bk_s.at[pl.ds(S + c * (S // 2), S // 2), :]),
                             (v_u, bv_s.at[c]), (wo_u, wo_s.at[c]))]

    w_first = w_copies(0)
    for cp in (w_first[:2] + [c_copy(n) for n in range(C_CHUNKS)]
               + [w_first[2], gw_copy, x_high, x_low]
               + [cp for p in range(1, H // 2) for cp in w_copies(p)]):
        cp.start()

    f_s[...] = _words(_dft(NFG, lambda n: n))
    inv = _words(_dft(NFG // 2, lambda n: 2 * (n & (W - 1)) + (n >> 6)).T * (1.0 / T))
    finv_s[0] = inv[:W // 2]
    finv_s[1] = inv[W // 2:]

    wq_rows, wk_rows, wv_rows = (
        slice(0, M // 2), slice(M // 2, (M + C) // 2), slice((M + C) // 2, M // 2 + C))

    def head_weights(pair, odd):
        half = pair & U32(0xFFFF0000) if odd else pair << 16
        return _words(pltpu.bitcast(half, F32))

    def load_wkv(w_ref, p, odd):
        w_ref[wk_rows, :] = head_weights(wuk_s[p], odd)
        w_ref[wv_rows, :] = head_weights(wuv_s[p], odd)

    def load_wq(p, odd):
        w_s[wq_rows, :] = head_weights(wq_s[p], odd)

    def up_project(dst, w_ref, w_rows, rows):
        dst[rows, :] = _words(_dot(_bf(ckv_s[rows, :]), _bf(w_ref[w_rows, :])))

    def gate_rows(h):
        rows = S // H
        gw = gw_s[...].astype(F32)
        acc = None
        for c in range(NCB):
            xw = x_s[pl.ds(pl.multiple_of(h * (rows // 2), rows // 2), rows // 2),
                     c * 128:(c + 1) * 128]
            term = _bf(xw).astype(F32) * gw[c:c + 1, :]
            acc = term if acc is None else acc + term
        z = jnp.sum(acc, axis=1, keepdims=True)
        g_s[pl.ds(pl.multiple_of(h * rows, rows), rows), :] = jax.nn.sigmoid(
            jnp.broadcast_to(z, (rows, 128)))

    def attention(h, k_ref, v_ref, plan, before_q, after_q):
        causal = (lax.broadcasted_iota(jnp.int32, (T, T), 1)
                  <= lax.broadcasted_iota(jnp.int32, (T, T), 0))
        val = {}
        for op, i in plan:
            n = (i + 1) * T
            if op == "q":
                before_q(i)
                q = _dot(_bf(x_s[_wblk(i), :]), _bf(w_s[wq_rows, :]))
                val[i] = (q * QSCALE).astype(BF16)
                if i == 0:
                    after_q()
                    gate_rows(h)
            elif op == "s":
                s = _dot_nt(val[i], _bf(k_ref[0:n // 2, :]))
                diag = jnp.where(causal, s[:, n - T:], -1e30)
                val[i] = jnp.concatenate([s[:, :n - T], diag], axis=1) if i else diag
            elif op == "c":
                p = jnp.exp2(val[i] - jnp.max(val[i], axis=1, keepdims=True))
                l = jnp.sum(p, axis=1, keepdims=True)
                o = _dot(p.astype(BF16), _bf(v_ref[0:n // 2, :]))
                r = pltpu.reciprocal(l, approx=True)
                val[i] = _words(o * (r * (2.0 - l * r)))
            elif op == "f":
                ctx_s[h, _wblk(i), :] = val.pop(i)
            elif op == "k":
                up_project(k_s, w_s, wk_rows, _wblk(i))
            else:
                up_project(v_s, w_s, wv_rows, _wblk(i))

    w_first[0].wait()
    w_first[1].wait()
    load_wkv(w0_s, 0, 0)
    load_wkv(w_s, 0, 1)

    def first_body(n, carry):
        c_copy(n).wait()
        up_project(k0_s, w0_s, wk_rows, c_rows(n))
        up_project(v0_s, w0_s, wv_rows, c_rows(n))
        up_project(k_s, w_s, wk_rows, c_rows(n))
        up_project(v_s, w_s, wv_rows, c_rows(n))
        return carry

    lax.fori_loop(0, C_CHUNKS, first_body, 0)
    w_first[2].wait()
    gw_copy.wait()
    load_wq(0, 0)
    x_high.wait()

    def pair_body(p, carry):
        @pl.when(p == W_SPLIT)
        def _():
            for later in range(W_SPLIT, H // 2):
                for cp in w_copies(later):
                    cp.wait()

        for odd in range(2):
            load_wkv(w_s, p, odd)
            attention(2 * p - 1 + odd, k_s, v_s, _REFILL_PLAN,
                      lambda i: None, lambda: load_wq(p, odd))
        return carry

    def edge_body(e, carry):
        def wait_x(i):
            if i == X_SPLIT - 1:
                pl.when(e == 0)(x_low.wait)

        attention(e * (H - 1), ctx_s.at[H + 1 - e], val_s.at[1 - e], _PLAIN_PLAN,
                  wait_x, lambda: None)

        @pl.when(e == 0)
        def _():
            for p in range(1, W_SPLIT):
                for cp in w_copies(p):
                    cp.wait()
            for cp in mix_copies:
                cp.start()
            load_wq(0, 1)
            lax.fori_loop(1, H // 2, pair_body, 0)

        return carry

    lax.fori_loop(0, 2, edge_body, 0)

    for cp in mix_copies:
        cp.wait()
    shift = shift_s[...].astype(F32)
    skip_w = d_s[...].astype(F32)
    for c in range(NCB):
        for t in range(4):
            par_s[c, t] = jnp.broadcast_to(shift[t:t + 1, c * 128:(c + 1) * 128], (8, 128))
        par_s[c, 4] = jnp.broadcast_to(skip_w[c:c + 1, :], (8, 128))

    def out_copy(c, lo, hi):
        rows = pl.ds(lo * W, (hi - lo) * W)
        return pltpu.make_async_copy(o_s.at[c, rows, :], out_u.at[rows, _lanes(c)], sems.at[5])

    def channel_body(c, carry):
        row0 = pl.multiple_of(zero_s[0] * 8, 8)

        def vregs(base, fg, j, n=1):
            return pl.ds(base + (fg * NB + j) * 8, 8 * n)

        def short_conv():
            before = jnp.zeros((8, 128), F32)
            n = KV_ROWS
            for j in range(S // n):
                k = _bf(bk_s[pl.ds(pl.multiple_of(S + c * (S // 2) + j * n // 2, 8), n // 2),
                             :]).astype(F32)
                ext = jnp.concatenate([before, k], axis=0)
                acc = None
                for t in range(4):
                    term = ext[8 - t:8 - t + n].reshape(n // 8, 8, 128) * par_s[c, t][None]
                    acc = term if acc is None else acc + term
                v = _bf(bv_s[c, j * n // 2:(j + 1) * n // 2, :]).astype(F32)
                bk_s[pl.ds(pl.multiple_of(row0 + j * n, 8), n), :] = pltpu.bitcast(
                    acc.reshape(n, 128) * v, U32)
                before = k[n - 8:]

        def kv_block(j):
            return pltpu.bitcast(bk_s[_blk(j), :], F32)

        def spectra():
            prev = None
            for d in range(NB):
                cur = _dot_nt(_bf(f_s[...]), h_s[_lanes(c), _blk(d)]).reshape(NFG, 2, 8, 128)
                re, im = cur[:, 0], cur[:, 1]
                if prev is not None:
                    re, im = re + prev[:, 1], im - prev[:, 0]
                for fg in range(NFG):
                    spec_s[vregs(O_HR, fg, d), :] = re[fg]
                    spec_s[vregs(O_HI, fg, d), :] = im[fg]
                prev = cur
            for j in range(NB):
                u = _dot(_bf(f_s[...]), kv_block(j).astype(BF16)).reshape(NFG, 2, 8, 128)
                for fg in range(NFG):
                    spec_s[vregs(O_UR, fg, j), :] = u[fg, 0]
                    spec_s[vregs(O_UI, fg, j), :] = u[fg, 1]

        def block_conv(fg, i):
            yr = yi = None
            for j in range(i + 1):
                hr = spec_s[vregs(O_HR, fg, i - j, 2), :].reshape(2, 8, 128)
                hi = spec_s[vregs(O_HI, fg, i - j, 2), :].reshape(2, 8, 128)
                ur = spec_s[vregs(O_UR, fg, j), :][None]
                ui = spec_s[vregs(O_UI, fg, j), :][None]
                tr, ti = hr * ur - hi * ui, hr * ui + hi * ur
                yr, yi = (tr, ti) if yr is None else (yr + tr, yi + ti)
            ur, ui = spec_s[vregs(O_UR, fg, i + 1), :], spec_s[vregs(O_UI, fg, i + 1), :]
            hr, hi = spec_s[vregs(O_HR, fg, 0), :], spec_s[vregs(O_HI, fg, 0), :]
            return ((yr[0], yi[0]),
                    (yr[1] + (hr * ur - hi * ui), yi[1] + (hr * ui + hi * ur)))

        def long_conv():
            for fg in range(NFG // 2):
                for i in range(0, NB, 2):
                    lo, hi = block_conv(fg, i), block_conv(fg + NFG // 2, i)
                    for n in range(2):
                        for odd in range(2):
                            pair = [p - q if odd else p + q for p, q in zip(lo[n], hi[n])]
                            row = pl.multiple_of(row0 + (i + n) * T + odd * W + fg * 8, 8)
                            spec_s[pl.ds(row, 8), :] = pltpu.bitcast(
                                jnp.concatenate(pair, axis=0).astype(BF16), F32)

        def inverse(i):
            even, odd = (
                pltpu.bitcast(_dot(_bf(finv_s[n]), _bf(spec_s[pl.ds(i * T + n * W, W), :]))
                              .astype(BF16).astype(F32), U32) for n in range(2))
            return _bf((even >> 16) | odd)

        def premix(i, a):
            g = g_s[_blk(i), :]
            skip = (kv_block(i).reshape(T // 8, 8, 128) * par_s[c, 4][None]).reshape(T, 128)
            gain = (1.0 - g) * _bf(x_s[_wblk(i), _lanes(c)]).astype(F32)
            return g * a + gain * skip, gain

        def finish(i, base, gain, y):
            o_s[c, _wblk(i), :] = _words(base + gain * y.astype(F32))

        y = {}
        for i in range(NB):
            if i == 12:
                long_conv()
            if i in (12, 13):
                for j in range((i - 12) * NB // 2, (i - 11) * NB // 2):
                    y[j] = inverse(j)
                    if j < 2:
                        finish(j, *premix(j, base_s[_blk(j), :]), y.pop(j))
                    elif j < i:
                        finish(j, base_s[_blk(j), :], gain_s[_blk(j), :], y.pop(j))
            ctx = jnp.concatenate([_bf(ctx_s[h, _wblk(i), :]) for h in range(H)], axis=1)
            a = _dot(ctx, _bf(wo_s[c]))
            if i == 0:
                bk_s[pl.ds(row0, 8), :] = pltpu.bitcast(a[0:8], U32)
                short_conv()
            if i == 2:
                spectra()
            rows = pl.ds(pl.multiple_of(row0 + i * T, 8), T)
            if i in y:
                finish(i, *premix(i, a), y.pop(i))
            elif i < 2:
                base_s[rows, :] = a
            else:
                base, gain = premix(i, a)
                gain_s[rows, :] = gain
                base_s[rows, :] = base
            if i == OUT_SPLIT - 1:
                out_copy(c, 0, OUT_SPLIT).start()
        out_copy(c, OUT_SPLIT, NB).start()
        return carry

    lax.fori_loop(0, NCB, channel_body, 0)
    for c in range(NCB):
        out_copy(c, 0, OUT_SPLIT).wait()
        out_copy(c, OUT_SPLIT, NB).wait()


@jax.jit
def pallas_gated_mix__compressed_kv_cla__ssm_conv_h3__prompt_kernel(
    A_x: jax.Array,
    A_c_kv: jax.Array,
    A_w_q: jax.Array,
    A_w_uk: jax.Array,
    A_w_uv: jax.Array,
    A_w_o: jax.Array,
    B_q: jax.Array,
    B_k: jax.Array,
    B_v: jax.Array,
    B_shift_k: jax.Array,
    B_ssm_k: jax.Array,
    B_ssm_D: jax.Array,
    gate_w: jax.Array,
):
    del B_q
    hbm = pl.BlockSpec(memory_space=pl.ANY)
    vmem = pltpu.VMEM
    out = pl.pallas_call(
        _kernel,
        out_shape=jax.ShapeDtypeStruct((S, M), BF16),
        in_specs=[hbm] * 12,
        out_specs=hbm,
        scratch_shapes=[
            vmem((S // 2, M), U32),
            vmem((S // 2, C), U32),
            vmem((H // 2, M, D), U32),
            vmem((H // 2, C, D), U32),
            vmem((H // 2, C, D), U32),
            vmem((NCB, H * D // 2, 128), U32),
            vmem((S + NCB * S // 2, 128), U32),
            vmem((NCB, S // 2, 128), U32),
            vmem((M, S), BF16),
            vmem((4, M), BF16),
            vmem((NCB, 128), BF16),
            vmem((NCB, 128), BF16),
            vmem((M // 2 + C, D), U32),
            vmem((M // 2 + C, D), U32),
            vmem((2, S // 2, D), U32),
            vmem((H + 2, S // 2, D), U32),
            vmem((S, 128), F32),
            vmem((T, T), U32),
            vmem((2, W // 2, T), U32),
            vmem((NCB, 8, 8, 128), F32),
            vmem((S, 128), F32),
            vmem((S, 128), F32),
            vmem((5 * S, 128), F32),
            vmem((NCB, S // 2, 128), U32),
            pltpu.SMEM((1,), jnp.int32),
            pltpu.SemaphoreType.DMA((9 + C_CHUNKS,)),
        ],
        compiler_params=pltpu.CompilerParams(vmem_limit_bytes=110 * 2 ** 20),
    )(A_x.reshape(S, M), A_c_kv.reshape(S, C), A_w_q, A_w_uk, A_w_uv,
      A_w_o.reshape(H * D, M), B_k.reshape(S, M), B_v.reshape(S, M),
      B_shift_k.T, B_ssm_k, B_ssm_D.reshape(NCB, 128), gate_w.reshape(NCB, 128))
    return out.reshape(1, S, M)
```

```python
import math

import jax
import jax.numpy as jnp
from jax import lax
import jax.experimental.pallas as pl
import jax.experimental.pallas.tpu as pltpu

S, M, C, H, D = 2048, 1024, 512, 32, 128
T = 128
W = T // 2
NB = S // T
NCB = M // 128
NFG = T // 16
F32, BF16, U32 = jnp.float32, jnp.bfloat16, jnp.uint32
QSCALE = D ** -0.5 * math.log2(math.e)

C_CHUNKS = 8
X_SPLIT = 8
W_SPLIT = 4
OUT_SPLIT = 14
KV_ROWS = 32
O_HR, O_HI, O_UR, O_UI = S, 2 * S, 3 * S, 4 * S


def _dot(a, b):
    return jnp.dot(a, b, preferred_element_type=F32)


def _dot_nt(a, b):
    return lax.dot_general(a, b, (((1,), (1,)), ((), ())), preferred_element_type=F32)


def _bf(words):
    return pltpu.bitcast(words, BF16)


def _words(val):
    return pltpu.bitcast(val.astype(BF16), U32)


def _blk(i):
    return slice(i * T, (i + 1) * T)


def _wblk(i):
    return slice(i * W, (i + 1) * W)


def _lanes(c):
    return pl.ds(pl.multiple_of(c * 128, 128), 128)


def _plan(delays, hurry=0):
    steps = []
    for n in range(NB):
        i = NB - 1 - n
        for pos, (op, delay) in enumerate(delays):
            t = NB - 1 - hurry if op in "qs" and i < hurry else n
            steps.append((t + delay, pos, n, op, i))
    return [step[3:] for step in sorted(steps)]


_REFILL_PLAN = _plan((("s", 2), ("f", 5), ("q", 0), ("k", 3), ("v", 3), ("c", 2)))
_PLAIN_PLAN = _plan((("q", 0), ("s", 1), ("f", 3), ("c", 2)), hurry=2)


def _dft(time, halves):
    def phasor(rows, step, first):
        r = lax.broadcasted_iota(jnp.int32, (rows, T), 0)
        n = time(lax.broadcasted_iota(jnp.int32, (rows, T), 1))
        ang = (((step * r + first) * n) & (4 * T - 1)).astype(F32) * (math.pi / (2 * T))
        return jnp.cos(ang), jnp.sin(ang)

    ca, sa = phasor(8, 4, 1)
    cb, sb = phasor(NFG * halves, 32, 0)
    rows = []
    for fg in range(NFG):
        turn = [(cb[r:r + 1, :], sb[r:r + 1, :]) for r in range(fg, NFG * halves, NFG)]
        rows += [ca * cf - sa * sf for cf, sf in turn]
        rows += [sa * cf + ca * sf for cf, sf in turn]
    return jnp.concatenate(rows, axis=0)


def _kernel(x_hbm, ckv_hbm, wq_hbm, wuk_hbm, wuv_hbm, wo_hbm, k_hbm, v_hbm,
            shift_hbm, h_hbm, d_hbm, gw_hbm, out_hbm,
            x_s, ckv_s, wq_s, wuk_s, wuv_s, wo_s, bk_s, bv_s, bx_s, h_s, shift_s, d_s, gw_s,
            w0_s, w_s, val_s, ctx_s, g_s, f_s, finv_s, par_s, base_s, gain_s, spec_s,
            o_s, zero_s, sems):
    x_u, ckv_u, wq_u, wuk_u, wuv_u, wo_u, k_u, v_u = (
        r.bitcast(U32) for r in
        (x_hbm, ckv_hbm, wq_hbm, wuk_hbm, wuv_hbm, wo_hbm, k_hbm, v_hbm))
    k_s, k0_s = ctx_s.at[H], ctx_s.at[H + 1]
    v_s, v0_s = val_s.at[0], val_s.at[1]
    zero_s[0] = 0

    def w_copies(p):
        kv, q = (0, 1) if p == 0 else (2, 2) if p < W_SPLIT else (3, 3)
        return [pltpu.make_async_copy(wuk_u.at[:, p, :], wuk_s.at[p], sems.at[kv]),
                pltpu.make_async_copy(wuv_u.at[:, p, :], wuv_s.at[p], sems.at[kv]),
                pltpu.make_async_copy(wq_u.at[:, p, :], wq_s.at[p], sems.at[q])]

    def row_copy(src, dst, rows, sem):
        return pltpu.make_async_copy(src.at[rows, :], dst.at[rows, :], sems.at[sem])

    def c_rows(n):
        rows = S // 2 // C_CHUNKS
        return pl.ds(pl.multiple_of(n * rows, rows), rows)

    def c_copy(n):
        return row_copy(ckv_u, ckv_s, c_rows(n), 9 + n)

    gw_copy = pltpu.make_async_copy(gw_hbm, gw_s, sems.at[6])
    x_high = row_copy(x_u, x_s, pl.ds(X_SPLIT * W, (NB - X_SPLIT) * W), 7)
    x_low = row_copy(x_u, x_s, pl.ds(0, X_SPLIT * W), 8)
    mix_copies = [pltpu.make_async_copy(src, dst, sems.at[4]) for src, dst in (
        (shift_hbm, shift_s), (d_hbm, d_s), (h_hbm, h_s))]
    for c in range(NCB):
        mix_copies += [
            pltpu.make_async_copy(src.at[:, pl.ds(c * 128, 128)], dst, sems.at[4])
            for src, dst in ((k_u, bk_s.at[pl.ds(S + c * (S // 2), S // 2), :]),
                             (v_u, bv_s.at[c]), (x_u, bx_s.at[c]), (wo_u, wo_s.at[c]))]

    w_first = w_copies(0)
    for cp in (w_first[:2] + [c_copy(n) for n in range(C_CHUNKS)]
               + [w_first[2], gw_copy, x_high, x_low]
               + [cp for p in range(1, H // 2) for cp in w_copies(p)]):
        cp.start()

    f_s[...] = _words(_dft(lambda n: n, 2))
    inv = _words(_dft(lambda n: 2 * (n & (W - 1)) + (n >> 6), 1).T * (1.0 / T))
    finv_s[0] = inv[:W // 2]
    finv_s[1] = inv[W // 2:]

    wq_rows, wk_rows, wv_rows = (
        slice(0, M // 2), slice(M // 2, (M + C) // 2), slice((M + C) // 2, M // 2 + C))

    def head_weights(pair, odd):
        half = pair & U32(0xFFFF0000) if odd else pair << 16
        return _words(pltpu.bitcast(half, F32))

    def load_wkv(w_ref, p, odd):
        w_ref[wk_rows, :] = head_weights(wuk_s[p], odd)
        w_ref[wv_rows, :] = head_weights(wuv_s[p], odd)

    def load_wq(p, odd):
        w_s[wq_rows, :] = head_weights(wq_s[p], odd)

    def up_project(dst, w_ref, w_rows, rows):
        dst[rows, :] = _words(_dot(_bf(ckv_s[rows, :]), _bf(w_ref[w_rows, :])))

    def gate_rows(h):
        rows = S // H
        gw = gw_s[...].astype(F32)
        acc = None
        for c in range(NCB):
            xw = x_s[pl.ds(pl.multiple_of(h * (rows // 2), rows // 2), rows // 2),
                     c * 128:(c + 1) * 128]
            term = _bf(xw).astype(F32) * gw[c:c + 1, :]
            acc = term if acc is None else acc + term
        z = jnp.sum(acc, axis=1, keepdims=True)
        g_s[pl.ds(pl.multiple_of(h * rows, rows), rows), :] = jax.nn.sigmoid(
            jnp.broadcast_to(z, (rows, 128)))

    def attention(h, k_ref, v_ref, plan, before_q, after_q):
        causal = (lax.broadcasted_iota(jnp.int32, (T, T), 1)
                  <= lax.broadcasted_iota(jnp.int32, (T, T), 0))
        val = {}
        for op, i in plan:
            n = (i + 1) * T
            if op == "q":
                before_q(i)
                q = _dot(_bf(x_s[_wblk(i), :]), _bf(w_s[wq_rows, :]))
                val[i] = (q * QSCALE).astype(BF16)
                if i == 0:
                    after_q()
                    gate_rows(h)
            elif op == "s":
                s = _dot_nt(val[i], _bf(k_ref[0:n // 2, :]))
                diag = jnp.where(causal, s[:, n - T:], -1e30)
                val[i] = jnp.concatenate([s[:, :n - T], diag], axis=1) if i else diag
            elif op == "c":
                p = jnp.exp2(val[i] - jnp.max(val[i], axis=1, keepdims=True))
                l = jnp.sum(p, axis=1, keepdims=True)
                o = _dot(p.astype(BF16), _bf(v_ref[0:n // 2, :]))
                r = pltpu.reciprocal(l, approx=True)
                val[i] = _words(o * (r * (2.0 - l * r)))
            elif op == "f":
                ctx_s[h, _wblk(i), :] = val.pop(i)
            elif op == "k":
                up_project(k_s, w_s, wk_rows, _wblk(i))
            else:
                up_project(v_s, w_s, wv_rows, _wblk(i))

    w_first[0].wait()
    w_first[1].wait()
    load_wkv(w0_s, 0, 0)
    load_wkv(w_s, 0, 1)

    def first_body(n, carry):
        c_copy(n).wait()
        up_project(k0_s, w0_s, wk_rows, c_rows(n))
        up_project(v0_s, w0_s, wv_rows, c_rows(n))
        up_project(k_s, w_s, wk_rows, c_rows(n))
        up_project(v_s, w_s, wv_rows, c_rows(n))
        return carry

    lax.fori_loop(0, C_CHUNKS, first_body, 0)
    w_first[2].wait()
    gw_copy.wait()
    load_wq(0, 0)
    x_high.wait()

    def pair_body(p, carry):
        @pl.when(p == W_SPLIT)
        def _():
            for later in range(W_SPLIT, H // 2):
                for cp in w_copies(later):
                    cp.wait()

        for odd in range(2):
            load_wkv(w_s, p, odd)
            attention(2 * p - 1 + odd, k_s, v_s, _REFILL_PLAN,
                      lambda i: None, lambda: load_wq(p, odd))
        return carry

    def edge_body(e, carry):
        def wait_x(i):
            if i == X_SPLIT - 1:
                pl.when(e == 0)(x_low.wait)

        attention(e * (H - 1), ctx_s.at[H + 1 - e], val_s.at[1 - e], _PLAIN_PLAN,
                  wait_x, lambda: None)

        @pl.when(e == 0)
        def _():
            for p in range(1, W_SPLIT):
                for cp in w_copies(p):
                    cp.wait()
            for cp in mix_copies:
                cp.start()
            load_wq(0, 1)
            lax.fori_loop(1, H // 2, pair_body, 0)

        return carry

    lax.fori_loop(0, 2, edge_body, 0)

    for cp in mix_copies:
        cp.wait()
    shift = shift_s[...].astype(F32)
    skip_w = d_s[...].astype(F32)
    for c in range(NCB):
        for t in range(4):
            par_s[c, t] = jnp.broadcast_to(shift[t:t + 1, c * 128:(c + 1) * 128], (8, 128))
        par_s[c, 4] = jnp.broadcast_to(skip_w[c:c + 1, :], (8, 128))

    def out_copy(c, lo, hi):
        rows = pl.ds(lo * T, (hi - lo) * T)
        return pltpu.make_async_copy(o_s.at[c, rows, :], out_hbm.at[rows, _lanes(c)], sems.at[5])

    def channel_body(c, carry):
        row0 = pl.multiple_of(zero_s[0] * 8, 8)

        def bins(base, fg, j, n=1):
            return pl.ds(base + (fg * NB + j) * 16, 16 * n)

        def short_conv():
            before = jnp.zeros((8, 128), F32)
            n = KV_ROWS
            for j in range(S // n):
                k = _bf(bk_s[pl.ds(pl.multiple_of(S + c * (S // 2) + j * n // 2, 8), n // 2),
                             :]).astype(F32)
                ext = jnp.concatenate([before, k], axis=0)
                acc = None
                for t in range(4):
                    term = ext[8 - t:8 - t + n].reshape(n // 8, 8, 128) * par_s[c, t][None]
                    acc = term if acc is None else acc + term
                v = _bf(bv_s[c, j * n // 2:(j + 1) * n // 2, :]).astype(F32)
                bk_s[pl.ds(pl.multiple_of(row0 + j * n, 8), n), :] = pltpu.bitcast(
                    acc.reshape(n, 128) * v, U32)
                before = k[n - 8:]

        def kv_block(j):
            return pltpu.bitcast(bk_s[_blk(j), :], F32)

        def spectra():
            def split(val):
                return [(val[fg * 32:fg * 32 + 16], val[fg * 32 + 16:fg * 32 + 32])
                        for fg in range(NFG)]

            prev = None
            for d in range(NB):
                cur = split(_dot_nt(_bf(f_s[...]), h_s[_lanes(c), _blk(d)]))
                for fg, (re, im) in enumerate(cur):
                    if prev is not None:
                        re, im = re + prev[fg][1], im - prev[fg][0]
                    spec_s[bins(O_HR, fg, d), :] = re
                    spec_s[bins(O_HI, fg, d), :] = im
                prev = cur
            for j in range(NB):
                cur = split(_dot(_bf(f_s[...]), kv_block(j).astype(BF16)))
                for fg, (re, im) in enumerate(cur):
                    spec_s[bins(O_UR, fg, j), :] = re
                    spec_s[bins(O_UI, fg, j), :] = im

        def product(fg, d, j, n):
            hr, hi = spec_s[bins(O_HR, fg, d, n), :], spec_s[bins(O_HI, fg, d, n), :]
            ur, ui = spec_s[bins(O_UR, fg, j), :], spec_s[bins(O_UI, fg, j), :]
            if n > 1:
                ur, ui = jnp.concatenate([ur] * n, axis=0), jnp.concatenate([ui] * n, axis=0)
            return hr * ur - hi * ui, hr * ui + hi * ur

        def long_conv():
            for fg in range(NFG):
                for i in range(0, NB, 2):
                    yr, yi = product(fg, i, 0, 2)
                    for j in range(1, i + 1):
                        tr, ti = product(fg, i - j, j, 2)
                        yr, yi = yr + tr, yi + ti
                    tr, ti = product(fg, 0, i + 1, 1)
                    for n, y in enumerate(((yr[:16], yi[:16]), (yr[16:] + tr, yi[16:] + ti))):
                        lo = jnp.concatenate([part[:8] for part in y], axis=0)
                        hi = jnp.concatenate([part[8:] for part in y], axis=0)
                        for odd, half in enumerate((lo + hi, lo - hi)):
                            row = pl.multiple_of(row0 + (i + n) * T + odd * W + fg * 8, 8)
                            spec_s[pl.ds(row, 8), :] = pltpu.bitcast(half.astype(BF16), F32)

        def inverse(i):
            even, odd = (
                pltpu.bitcast(_dot(_bf(finv_s[n]), _bf(spec_s[pl.ds(i * T + n * W, W), :]))
                              .astype(BF16).astype(F32), U32) for n in range(2))
            return _bf((even >> 16) | odd)

        def premix(i, a):
            g = g_s[_blk(i), :]
            skip = (kv_block(i).reshape(T // 8, 8, 128) * par_s[c, 4][None]).reshape(T, 128)
            gain = (1.0 - g) * _bf(bx_s[c, _wblk(i), :]).astype(F32)
            return g * a + gain * skip, gain

        def finish(i, base, gain, y):
            o_s[c, _blk(i), :] = (base + gain * y.astype(F32)).astype(BF16)

        y = {}
        for i in range(NB):
            if i == 12:
                long_conv()
            if i in (12, 13):
                for j in range((i - 12) * NB // 2, (i - 11) * NB // 2):
                    y[j] = inverse(j)
                    if j < 2:
                        finish(j, *premix(j, base_s[_blk(j), :]), y.pop(j))
                    elif j < i:
                        finish(j, base_s[_blk(j), :], gain_s[_blk(j), :], y.pop(j))
            ctx = jnp.concatenate([_bf(ctx_s[h, _wblk(i), :]) for h in range(H)], axis=1)
            a = _dot(ctx, _bf(wo_s[c]))
            if i == 0:
                bk_s[pl.ds(row0, 8), :] = pltpu.bitcast(a[0:8], U32)
                short_conv()
            if i == 2:
                spectra()
            rows = pl.ds(pl.multiple_of(row0 + i * T, 8), T)
            if i in y:
                finish(i, *premix(i, a), y.pop(i))
            elif i < 2:
                base_s[rows, :] = a
            else:
                base, gain = premix(i, a)
                gain_s[rows, :] = gain
                base_s[rows, :] = base
            if i == OUT_SPLIT - 1:
                out_copy(c, 0, OUT_SPLIT).start()
        out_copy(c, OUT_SPLIT, NB).start()
        return carry

    lax.fori_loop(0, NCB, channel_body, 0)
    for c in range(NCB):
        out_copy(c, 0, OUT_SPLIT).wait()
        out_copy(c, OUT_SPLIT, NB).wait()


@jax.jit
def pallas_gated_mix__compressed_kv_cla__ssm_conv_h3__prompt_kernel(
    A_x: jax.Array,
    A_c_kv: jax.Array,
    A_w_q: jax.Array,
    A_w_uk: jax.Array,
    A_w_uv: jax.Array,
    A_w_o: jax.Array,
    B_q: jax.Array,
    B_k: jax.Array,
    B_v: jax.Array,
    B_shift_k: jax.Array,
    B_ssm_k: jax.Array,
    B_ssm_D: jax.Array,
    gate_w: jax.Array,
):
    del B_q
    hbm = pl.BlockSpec(memory_space=pl.ANY)
    vmem = pltpu.VMEM
    out = pl.pallas_call(
        _kernel,
        out_shape=jax.ShapeDtypeStruct((S, M), BF16),
        in_specs=[hbm] * 12,
        out_specs=hbm,
        scratch_shapes=[
            vmem((S // 2, M), U32),
            vmem((S // 2, C), U32),
            vmem((H // 2, M, D), U32),
            vmem((H // 2, C, D), U32),
            vmem((H // 2, C, D), U32),
            vmem((NCB, H * D // 2, 128), U32),
            vmem((S + NCB * S // 2, 128), U32),
            vmem((NCB, S // 2, 128), U32),
            vmem((NCB, S // 2, 128), U32),
            vmem((M, S), BF16),
            vmem((4, M), BF16),
            vmem((NCB, 128), BF16),
            vmem((NCB, 128), BF16),
            vmem((M // 2 + C, D), U32),
            vmem((M // 2 + C, D), U32),
            vmem((2, S // 2, D), U32),
            vmem((H + 2, S // 2, D), U32),
            vmem((S, 128), F32),
            vmem((T, T), U32),
            vmem((2, W // 2, T), U32),
            vmem((NCB, 8, 8, 128), F32),
            vmem((S, 128), F32),
            vmem((S, 128), F32),
            vmem((5 * S, 128), F32),
            vmem((NCB, S, 128), BF16),
            pltpu.SMEM((1,), jnp.int32),
            pltpu.SemaphoreType.DMA((9 + C_CHUNKS,)),
        ],
        compiler_params=pltpu.CompilerParams(vmem_limit_bytes=110 * 2 ** 20),
    )(A_x.reshape(S, M), A_c_kv.reshape(S, C), A_w_q, A_w_uk, A_w_uv,
      A_w_o.reshape(H * D, M), B_k.reshape(S, M), B_v.reshape(S, M),
      B_shift_k.T, B_ssm_k, B_ssm_D.reshape(NCB, 128), gate_w.reshape(NCB, 128))
    return out.reshape(1, S, M)
```
